```python
import os as _os
_os.environ.setdefault("JAX_PLATFORMS", "cpu")
import jax
import jax.numpy as jnp

def _softmax(x, axis=-1):
    return jax.nn.softmax(x, axis=axis)
def _gelu(x):
    return jax.nn.gelu(x, approximate=True)
def _silu(x):
    return jax.nn.silu(x)
def _sigmoid(x):
    return jax.nn.sigmoid(x)
def _layernorm(x, axis=-1, eps=1e-5):
    m = jnp.mean(x, axis=axis, keepdims=True)
    v = jnp.var(x, axis=axis, keepdims=True)
    return (x - m) / jnp.sqrt(v + eps)
def _scatter_add(tgt, idx, src, axis=0):
    return tgt.at[idx].add(src)
def _segment_sum(src, seg, n):
    return jax.ops.segment_sum(src, seg, n)
class _Rng:
    def __init__(self, key):
        self._k = key
    def _next(self):
        self._k, sub = jax.random.split(self._k)
        return sub
    def normal(self, shape):
        return jax.random.normal(self._next(), shape, dtype=jnp.bfloat16)
    def randint(self, lo, hi, shape):
        return jax.random.randint(self._next(), shape, lo, hi, dtype=jnp.int32)
    def uniform(self, shape, lo=0.0, hi=1.0):
        return jax.random.uniform(self._next(), shape, jnp.bfloat16, lo, hi)
    def permutation(self, n):
        return jax.random.permutation(self._next(), n)


kernel_name = 'parallel_sum__sliding_block__moe_arch_mod__prompt'

def setup_inputs():
    _rng = _Rng(jax.random.key(int.from_bytes(__import__("os").urandom(4), "little")))
    _w = (lambda a: (lambda t: t.astype(jnp.bfloat16) if jnp.issubdtype(t.dtype, jnp.floating) else t)(jnp.asarray(a)))
    def _A_setup():
        B, S, D = 1, 2048, 512
        return {
            "x": _w((lambda *s: _rng.normal(s) * 0.05)(B, S, D)),
            "wqkv": _w((lambda *s: _rng.normal(s) * 0.05)(D, 3 * D)),
            "wo": _w((lambda *s: _rng.normal(s) * 0.05)(D, D)),
        }
    _A_in = _A_setup()

    def _B_setup():
        B, S, D, F, C = 1, 2048, 512, 1376, 1
        return {
            "x": _w((lambda *s: _rng.normal(s) * 0.05)(B, S, D)),
            "w_r": _w((lambda *s: _rng.normal(s) * 0.05)(D)),
            "w_gate": _w((lambda *s: _rng.normal(s) * 0.05)(D, F)),
            "w_up": _w((lambda *s: _rng.normal(s) * 0.05)(D, F)),
            "w_down": _w((lambda *s: _rng.normal(s) * 0.05)(F, D)),
        }
    _B_in = _B_setup()

    return {
        "A_x": _A_in["x"],
        "A_wqkv": _A_in["wqkv"],
        "A_wo": _A_in["wo"],
        "B_x": _B_in["x"],
        "B_w_r": _B_in["w_r"],
        "B_w_gate": _B_in["w_gate"],
        "B_w_up": _B_in["w_up"],
        "B_w_down": _B_in["w_down"],
    }

def reference(A_x, A_wqkv, A_wo, B_x, B_w_r, B_w_gate, B_w_up, B_w_down):
    def _A_ref(x, wqkv, wo):
        B, S, D = x.shape
        H = 32; Dh = D // H; W = 256
        qkv = (lambda x, *d: x.transpose(*d))((x @ wqkv).reshape(B, S, 3, H, Dh), 2, 0, 3, 1, 4)
        q, k, v = qkv[0], qkv[1], qkv[2]
        scores = jnp.einsum("bhqd,bhkd->bhqk", q, k) * (Dh ** -0.5)
        idx = jnp.arange(S)
        mask = (idx[:, None] - idx[None, :] >= 0) & (idx[:, None] - idx[None, :] < W)
        scores = jnp.where(mask[None, None], scores, -1e9)
        p = _softmax(scores, axis=-1)
        o = jnp.einsum("bhqk,bhkd->bhqd", p, v)
        return (lambda x, *d: x.transpose(*d))(o, 0, 2, 1, 3).reshape(B, S, D) @ wo

    def _B_ref(x, w_r, w_gate, w_up, w_down):
        B, S, D = x.shape
        C = 1
        r = x @ w_r
        idx = jnp.argsort(-r, axis=-1)[:, :C]
        idx_e = jnp.repeat(idx.reshape(B, C, 1), D, axis=2)
        x_sel = jnp.take_along_axis(x, idx_e, axis=1)
        g = _silu(x_sel @ w_gate)
        u = x_sel @ w_up
        y = (g * u) @ w_down
        r_sel = _sigmoid(jnp.take_along_axis(r, idx, axis=1))
        y = y * r_sel.reshape(B, C, 1)
        b_off = (jnp.arange(B) * S).reshape(B, 1)
        flat_idx = (idx + b_off).reshape(B * C)
        zero = (x * 0.0).reshape(B * S, D)
        upd = _scatter_add(zero, flat_idx, y.reshape(B * C, D), axis=0)
        return x + upd.reshape(B, S, D)

    x = A_x
    xn = _layernorm(x, axis=-1)
    return x + _A_ref(xn, A_wqkv, A_wo) + _B_ref(xn, B_w_r, B_w_gate, B_w_up, B_w_down)
```

```python
import jax
import jax.numpy as jnp
import numpy as np
from jax import lax
import jax.experimental.pallas as pl
import jax.experimental.pallas.tpu as pltpu

S = 2048
D = 512
H = 32
DH = 16
F = 1376
T = 128
NT = S // T
NG = 4
TP = 2
NEG = -1e30
QSCALE = (DH ** -0.5) * 1.4426950408889634
BF = jnp.bfloat16
F32 = jnp.float32
EPS_BF = float(np.asarray(1e-5, dtype=jnp.bfloat16).astype(np.float32))

ORDER_FIRST = ("ln q0 q1 s0 q2 s1 a0 q3 s2 q4 s3 pw a1 q5 s4 q6 s5 a2 q7 s6 q8 s7 a3 q9 s8 q10 s9 q11 s10 "
               "q12 s11 a5 q13 s12 q14 a4 s13 q15 s14 a6 pk0 pqv0 s15 a7 pk1 pqv1 wo")
ORDER_LOOP = ("ln q0 q1 s0 q2 s1 a0 q3 s2 q4 s3 q5 a1 s4 q6 s5 q7 s6 q8 s7 a2 a3 q9 s8 q10 s9 q11 s10 "
              "q12 s11 q13 s12 q14 s13 q15 a4 s14 pk0 s15 a6 a7 a5 wo0 pqv wo1 pk1")
ORDER_LAST = ("q0 fg q1 s0 q2 s1 fu q3 s2 q4 s3 q5 a0 s4 q6 s5 a1 a2 q7 s6 q8 s7 a3 q9 s8 fa q10 s9 q11 s10 "
              "q12 s11 q13 s12 a5 q14 s13 a6 a4 fb q15 s14 fc s15 a7 wo0 fd wo1")


def _nt(a, b):
    return lax.dot_general(a, b, (((1,), (1,)), ((), ())), preferred_element_type=F32)


def _nn(a, b):
    return jnp.dot(a, b, preferred_element_type=F32)


def _rb(v):
    return v.astype(BF).astype(F32)


def _kernel(x_hbm, wqkv_hbm, wo_hbm, wr_hbm, wg_hbm, wu_hbm, wd_hbm, out_hbm,
            x_v, wq_v, wk_v, wv_v, wo_v, wr_v, wg_v, wu_v, wd_v,
            wop_v, wgn_v, wun_v, wqvt_v, k_v, vt_v, xn_v, qt_v, out_v, r_v, s0_v, s1_v,
            sem_x, sem_w, sem_o):
    def x_copy(c):
        return pltpu.make_async_copy(x_hbm.at[pl.ds(c * T, T)], x_v.at[pl.ds(c * T, T)], sem_x.at[c])

    def out_copy(c):
        return pltpu.make_async_copy(out_v.at[pl.ds(c * T, T)], out_hbm.at[pl.ds(c * T, T)], sem_o.at[c])

    c_wq = pltpu.make_async_copy(wqkv_hbm.at[:, pl.ds(0, D)], wq_v, sem_w.at[0])
    c_wk = pltpu.make_async_copy(wqkv_hbm.at[:, pl.ds(D, D)], wk_v, sem_w.at[7])
    c_wv = pltpu.make_async_copy(wqkv_hbm.at[:, pl.ds(2 * D, D)], wv_v, sem_w.at[8])
    c_wr = pltpu.make_async_copy(wr_hbm, wr_v, sem_w.at[1])
    c_wo = pltpu.make_async_copy(wo_hbm, wo_v, sem_w.at[2])
    c_wg = pltpu.make_async_copy(wg_hbm, wg_v, sem_w.at[3])
    c_wu = pltpu.make_async_copy(wu_hbm, wu_v, sem_w.at[4])
    c_wd = pltpu.make_async_copy(wd_hbm, wd_v, sem_w.at[5])

    x_copy(0).start()
    c_wk.start()

    k_v[:, 0:2 * T, :] = jnp.zeros((NG, 2 * T, T), BF)
    vt_v[0:2] = jnp.zeros((2, D, T), BF)

    s_refs = (s0_v, s1_v)
    ffn = {}

    def row0(u):
        return u * T if isinstance(u, int) else pl.multiple_of(u * T, T)

    def ln(u, wait):
        r0 = row0(u)
        if wait:
            x_copy(u).wait()
        xf = x_v[pl.ds(r0, T), :].astype(F32)
        mean = jnp.mean(xf, axis=-1, keepdims=True)
        cen = xf - mean
        var = jnp.mean(cen * cen, axis=-1, keepdims=True)
        m_b = _rb(mean)
        v_b = _rb(var)
        s_b = _rb(jnp.sqrt(_rb(v_b + EPS_BF)))
        xn = (_rb(xf - m_b) / s_b).astype(BF)
        xn_v[pl.ds(r0, T), :] = xn

    def proj_k(u, nt):
        r0 = row0(u)
        xn = xn_v[pl.ds(r0, nt * T), :]
        k = _nn(xn, wk_v[...]).astype(BF)
        for g in range(NG):
            k_v[g, pl.ds(r0 + 2 * T, nt * T), :] = k[:, g * 128:(g + 1) * 128]

    def store_qt(u, q):
        qb = (q * QSCALE).astype(BF)
        parts = []
        for h in range(H):
            blk = qb[h * DH:(h + 1) * DH]
            parts.append(pltpu.roll(blk, 64, axis=1) if h % 2 else blk)
        qb = jnp.concatenate(parts, axis=0)
        hrow = lax.broadcasted_iota(jnp.int32, (D, T), 0) >> 4
        half = lax.broadcasted_iota(jnp.int32, (D, T), 1) >> 6
        keep0 = ((hrow ^ half) & 1) == 0
        zero = jnp.zeros((D, T), BF)
        qt_v[u, 0] = jnp.where(keep0, qb, zero)
        qt_v[u, 1] = jnp.where(keep0, zero, qb)

    def proj_qv(u, nt):
        xn = xn_v[pl.ds(row0(u), nt * T), :]
        t = _nt(wqvt_v[...], xn)
        for j in range(nt):
            tj = t[:, j * T:(j + 1) * T]
            store_qt(u + j, tj[0:D])
            vt_v[u + 2 + j] = tj[D:2 * D].astype(BF)
            r_v[u + j] = _rb(tj[2 * D:2 * D + 8])

    def transpose_w(w_ref, j):
        for i in range(NG):
            wqvt_v[j * D + i * 128: j * D + (i + 1) * 128, :] = w_ref[:, i * 128:(i + 1) * 128].T

    def qk_phase(u, r0, n, nblk, tri_a, tri_e, slot):
        g, par = divmod(n, 2)
        zero = jnp.zeros((16, 128), BF)
        tiles = []
        for p in range(4):
            both = qt_v[u, par, (g * 8 + 2 * p) * 16:(g * 8 + 2 * p + 2) * 16, :]
            rows = [zero] * (2 * p) + [both] + [zero] * (6 - 2 * p)
            tiles.append(jnp.concatenate(rows, axis=0))
        qm = jnp.concatenate(tiles, axis=1)
        skip = 5 - nblk
        ks = r0 + 64 * par + 64 * skip
        kb = k_v[g, pl.ds(ks, 64 * nblk), :]
        s = _nn(kb, qm)
        blocks = [s[64 * b:64 * (b + 1)] for b in range(nblk)]
        lsl = [slice(p * 128, (p + 1) * 128) for p in range(4)]
        if nblk == 5:
            comb = jnp.concatenate([jnp.where(tri_a, blocks[0][:, l_], blocks[4][:, l_]) for l_ in lsl], axis=1)
            mids = blocks[1:4]
        else:
            comb = jnp.concatenate([jnp.where(tri_e, blocks[-1][:, l_], NEG) for l_ in lsl], axis=1)
            mids = blocks[:-1]
        s_ref = s_refs[slot % 2]
        s_ref[0:64, :] = comb
        m = comb
        for i, b in enumerate(mids):
            s_ref[64 * (i + 1):64 * (i + 2), :] = b
            m = jnp.maximum(m, b)
        return jnp.max(m, axis=0, keepdims=True)

    def smpv_phase(u, n, nblk, m, tri_a, slot):
        g, par = divmod(n, 2)
        s_ref = s_refs[slot % 2]
        skip = 5 - nblk
        outs = []
        for p in range(4):
            ls = slice(p * 128, (p + 1) * 128)
            mp = m[:, ls]
            hrow = (g * 8 + 2 * p) * DH
            if nblk == 5:
                ex = lambda b: jnp.exp2(s_ref[64 * b:64 * (b + 1), ls] - mp)
                z = jnp.zeros((64, 128), F32)
                pc = ex(0)
                l = pc
                pa = jnp.where(tri_a, pc, 0.0)
                pe = jnp.where(tri_a, 0.0, pc)
                if par == 0:
                    b1 = ex(1)
                    l = l + b1
                    t0 = jnp.concatenate([pa, b1], axis=0).astype(BF)
                    o = _nn(vt_v[u, hrow:hrow + 32, :], t0)
                    b2 = ex(2)
                    b3 = ex(3)
                    l = l + b2 + b3
                    t1 = jnp.concatenate([b2, b3], axis=0).astype(BF)
                    o = o + _nn(vt_v[u + 1, hrow:hrow + 32, :], t1)
                    t2 = jnp.concatenate([pe, z], axis=0).astype(BF)
                    o = o + _nn(vt_v[u + 2, hrow:hrow + 32, :], t2)
                else:
                    t0 = jnp.concatenate([z, pa], axis=0).astype(BF)
                    o = _nn(vt_v[u, hrow:hrow + 32, :], t0)
                    b1 = ex(1)
                    b2 = ex(2)
                    l = l + b1 + b2
                    t1 = jnp.concatenate([b1, b2], axis=0).astype(BF)
                    o = o + _nn(vt_v[u + 1, hrow:hrow + 32, :], t1)
                    b3 = ex(3)
                    l = l + b3
                    t2 = jnp.concatenate([b3, pe], axis=0).astype(BF)
                    o = o + _nn(vt_v[u + 2, hrow:hrow + 32, :], t2)
                l = jnp.sum(l, axis=0, keepdims=True)
            else:
                ps = [jnp.exp2(s_ref[64 * b:64 * (b + 1), ls] - mp) for b in range(nblk)]
                l = ps[0]
                for b in ps[1:]:
                    l = l + b
                l = jnp.sum(l, axis=0, keepdims=True)
                z = jnp.zeros((64, 128), F32)
                seq = ps[1:] + [ps[0]]
                al = [z] * skip + seq + [z] if par == 0 else [z] * (1 + skip) + seq
                j0 = skip // 2 if par == 0 else (1 + skip) // 2
                P = jnp.concatenate(al[2 * j0:], axis=0).astype(BF)
                vwin = jnp.concatenate([vt_v[u + j, hrow:hrow + 32, :] for j in range(j0, 3)], axis=1)
                o = _nn(vwin, P)
            r = pl.reciprocal(l, approx=True)
            r = r * (2.0 - l * r)
            outs.append(o * r)
        return outs

    def step(u0, nblks, nxt, order):
        lane = lax.broadcasted_iota(jnp.int32, (64, 128), 1)
        row = lax.broadcasted_iota(jnp.int32, (64, 128), 0)
        qi = lane & 63
        tri_a = row > qi
        tri_e = row <= qi
        lane_lo16 = lax.broadcasted_iota(jnp.int32, (16, 128), 1) < 64
        ms, res, ots = {}, {}, {}

        for tk in order.split():
            kind = tk.rstrip('0123456789')
            num = int(tk[len(kind):]) if len(tk) > len(kind) else None
            if kind == 'ln':
                if nxt:
                    for j in range(TP):
                        ln(u0 + TP + j, False)
            elif kind == 'pk':
                if nxt:
                    proj_k(u0 + TP, TP) if num is None else proj_k(u0 + TP + num, 1)
            elif kind == 'pqv':
                if nxt:
                    proj_qv(u0 + TP, TP) if num is None else proj_qv(u0 + TP + num, 1)
            elif kind == 'q':
                j, n = divmod(num, 8)
                ms[num] = qk_phase(u0 + j, row0(u0 + j), n, nblks[j][n % 2], tri_a, tri_e, num)
            elif kind == 's':
                j, n = divmod(num, 8)
                res[num] = smpv_phase(u0 + j, n, nblks[j][n % 2], ms[num], tri_a, num)
            elif kind == 'pw':
                for h in range(H):
                    dst = (h % 2) * (D // 2) + (h // 2) * DH
                    wop_v[dst:dst + DH, :] = wo_v[h * DH:(h + 1) * DH, :]
            elif kind == 'a':
                pe_, po_ = [], []
                for p in range(4):
                    re_, ro_ = res[2 * num][p], res[2 * num + 1][p]
                    pe_.append(jnp.where(lane_lo16, re_[0:16], ro_[0:16]))
                    po_.append(jnp.where(lane_lo16, ro_[16:32], re_[16:32]))
                ots[num] = (jnp.concatenate(pe_, axis=0).astype(BF), jnp.concatenate(po_, axis=0).astype(BF))
            elif kind == 'wo':
                js = range(TP) if num is None else [num]

                def lhs(parity):
                    return jnp.concatenate(
                        [jnp.concatenate([ots[NG * j + g][parity] for g in range(NG)], axis=0).T for j in js], axis=0)
                ae = _nn(lhs(0), wop_v[0:D // 2])
                ao = _nn(lhs(1), wop_v[D // 2:D])
                sw = []
                for i_ in range(len(js)):
                    sw += [ao[i_ * T + 64:(i_ + 1) * T], ao[i_ * T:i_ * T + 64]]
                a = ae + jnp.concatenate(sw, axis=0)
                for i_, j in enumerate(js):
                    r0 = row0(u0 + j)
                    resid = (x_v[pl.ds(r0, T), :].astype(F32) + xn_v[pl.ds(r0, T), :].astype(F32)
                             + a[i_ * T:(i_ + 1) * T])
                    if 'y' in ffn:
                        rows_abs = lax.broadcasted_iota(jnp.int32, (T, D), 0) + (u0 + j) * T
                        resid = resid + jnp.where(rows_abs == ffn['idx'], ffn['y'][0:1, :], 0.0)
                    out_v[pl.ds(r0, T), :] = resid.astype(BF)
                    out_copy(u0 + j).start()
            elif kind in ('fg', 'fu'):
                src, dst = (wg_v, wgn_v) if kind == 'fg' else (wu_v, wun_v)
                for i in range(pl.cdiv(F, 128)):
                    n_ = min(128, F - i * 128)
                    dst[:, i * 128:i * 128 + n_] = src[i * 128:i * 128 + n_, :].T
            elif kind == 'fa':
                r = r_v[...][:, 0, :]
                tok = (lax.broadcasted_iota(jnp.int32, (NT, 128), 0) * 128
                       + lax.broadcasted_iota(jnp.int32, (NT, 128), 1))
                rmax = jnp.max(jnp.max(r, axis=1, keepdims=True), axis=0, keepdims=True)
                idx = jnp.minimum(jnp.min(jnp.where(r == rmax, tok, S)), S - 1)
                blk = pl.multiple_of((idx // 16) * 16, 16)
                sel = (lax.broadcasted_iota(jnp.int32, (16, D), 0) + blk) == idx
                xrow = jnp.sum(jnp.where(sel, xn_v[pl.ds(blk, 16), :].astype(F32), 0.0), axis=0, keepdims=True)
                ffn.update(idx=idx, blk=blk, rmax=rmax, xs=jnp.broadcast_to(xrow, (16, D)).astype(BF))
            elif kind == 'fb':
                ffn['gp'] = _rb(_nn(ffn['xs'], wgn_v[...]))
                ffn['up'] = _rb(_nn(ffn['xs'], wun_v[...]))
            elif kind == 'fc':
                gp = ffn['gp']
                hh = (_rb(gp * jax.nn.sigmoid(gp)) * ffn['up']).astype(BF)
                y = _rb(_nn(hh, wd_v[...]))
                ffn['y'] = _rb(y * _rb(jax.nn.sigmoid(ffn['rmax'])))
            elif kind == 'fd':
                pblk = pl.multiple_of(jnp.minimum(ffn['blk'], u0 * T - 16), 16)
                psel = (lax.broadcasted_iota(jnp.int32, (16, D), 0) + pblk) == ffn['idx']
                cur = out_v[pl.ds(pblk, 16), :].astype(F32)
                out_v[pl.ds(pblk, 16), :] = jnp.where(psel, cur + ffn['y'], cur).astype(BF)
                patch = pltpu.make_async_copy(out_v.at[pl.ds(pblk, 16)], out_hbm.at[pl.ds(pblk, 16)], sem_w.at[6])
                patch.start()
                ffn['patch'] = patch
            else:
                raise ValueError(tk)

    x_copy(0).wait()
    c_wq.start()
    c_wv.start()
    c_wr.start()
    x_copy(1).start()
    ln(0, False)
    c_wk.wait()
    c_wo.start()
    for c in range(2, 2 + TP):
        x_copy(c).start()
    proj_k(0, 1)
    ln(1, True)
    proj_k(1, 1)
    c_wq.wait()
    transpose_w(wq_v, 0)
    c_wv.wait()
    c_wr.wait()
    transpose_w(wv_v, 1)
    wqvt_v[2 * D:2 * D + 16, :] = jnp.broadcast_to(wr_v[...].reshape(1, D), (16, D))
    for c in range(2 + TP, NT):
        x_copy(c).start()
    proj_qv(0, TP)
    c_wo.wait()
    for c in range(2, 2 + TP):
        x_copy(c).wait()

    step(0, [(1, 2), (3, 4)], True, ORDER_FIRST)
    c_wg.start()
    c_wu.start()
    c_wd.start()
    for c in range(2 + TP, NT):
        x_copy(c).wait()
    full = [(5, 5)] * TP

    def body(i, carry):
        step((i + 1) * TP, full, True, ORDER_LOOP)
        return carry
    lax.fori_loop(0, NT // TP - 2, body, 0)

    c_wg.wait()
    c_wu.wait()
    c_wd.wait()
    for c in range(NT - TP):
        out_copy(c).wait()
    step(NT - TP, full, False, ORDER_LAST)
    for j in range(TP):
        out_copy(NT - TP + j).wait()
    ffn['patch'].wait()


@jax.jit
def pallas_parallel_sum__sliding_block__moe_arch_mod__prompt_kernel(
    A_x: jax.Array,
    A_wqkv: jax.Array,
    A_wo: jax.Array,
    B_x: jax.Array,
    B_w_r: jax.Array,
    B_w_gate: jax.Array,
    B_w_up: jax.Array,
    B_w_down: jax.Array,
):
    del B_x
    hbm = pl.BlockSpec(memory_space=pltpu.HBM)
    out = pl.pallas_call(
        _kernel,
        out_shape=jax.ShapeDtypeStruct((S, D), BF),
        in_specs=[hbm] * 7,
        out_specs=hbm,
        scratch_shapes=[
            pltpu.VMEM((S, D), BF),
            pltpu.VMEM((D, D), BF),
            pltpu.VMEM((D, D), BF),
            pltpu.VMEM((D, D), BF),
            pltpu.VMEM((D, D), BF),
            pltpu.VMEM((D,), BF),
            pltpu.VMEM((F, D), BF),
            pltpu.VMEM((F, D), BF),
            pltpu.VMEM((F, D), BF),
            pltpu.VMEM((D, D), BF),
            pltpu.VMEM((D, F), BF),
            pltpu.VMEM((D, F), BF),
            pltpu.VMEM((2 * D + 16, D), BF),
            pltpu.VMEM((NG, S + 2 * T, 128), BF),
            pltpu.VMEM((NT + 2, D, T), BF),
            pltpu.VMEM((S, D), BF),
            pltpu.VMEM((NT, 2, D, T), BF),
            pltpu.VMEM((S, D), BF),
            pltpu.VMEM((NT, 8, T), F32),
            pltpu.VMEM((256, 512), F32),
            pltpu.VMEM((256, 512), F32),
            pltpu.SemaphoreType.DMA((NT,)),
            pltpu.SemaphoreType.DMA((9,)),
            pltpu.SemaphoreType.DMA((NT,)),
        ],
        compiler_params=pltpu.CompilerParams(
            vmem_limit_bytes=64 * 1024 * 1024,
            flags={'XLA_TPU_EVENLY_DISTRIBUTE_CRITICAL_NODES': True},
        ),
    )(A_x.reshape(S, D), A_wqkv, A_wo, B_w_r, B_w_gate.T, B_w_up.T, B_w_down)
    return out.reshape(1, S, D)
```

```python
import jax
import jax.numpy as jnp
import numpy as np
from jax import lax
import jax.experimental.pallas as pl
import jax.experimental.pallas.tpu as pltpu

S = 2048
D = 512
H = 32
DH = 16
F = 1376
T = 128
NT = S // T
NG = 4
TP = 2
NEG = -1e30
QSCALE = (DH ** -0.5) * 1.4426950408889634
BF = jnp.bfloat16
F32 = jnp.float32
EPS_BF = float(np.asarray(1e-5, dtype=jnp.bfloat16).astype(np.float32))

ORDER_FIRST = ("ln q0 q1 s0 q2 s1 a0 q3 s2 q4 s3 pw a1 q5 s4 q6 s5 a2 q7 s6 q8 s7 a3 q9 s8 q10 s9 q11 s10 "
               "q12 s11 a5 q13 s12 q14 a4 s13 q15 s14 a6 pk0 pqv0 s15 a7 pk1 pqv1 wo")
ORDER_LOOP = ("ln q0 q1 s0 q2 s1 a0 q3 s2 q4 s3 q5 a1 s4 q6 s5 q7 s6 q8 s7 a2 a3 q9 s8 q10 s9 q11 s10 "
              "q12 s11 q13 s12 q14 s13 q15 a4 s14 pk0 s15 a6 a7 a5 wo0 pqv wo1 pk1")
ORDER_LAST = ("q0 fg q1 s0 q2 s1 fu q3 s2 q4 s3 q5 a0 s4 q6 s5 a1 a2 q7 s6 q8 s7 a3 q9 s8 fa q10 s9 q11 s10 "
              "q12 s11 q13 s12 a5 q14 s13 a6 a4 fb q15 s14 fc s15 a7 wo0 fd wo1")


def _nt(a, b):
    return lax.dot_general(a, b, (((1,), (1,)), ((), ())), preferred_element_type=F32)


def _nn(a, b):
    return jnp.dot(a, b, preferred_element_type=F32)


def _rb(v):
    return v.astype(BF).astype(F32)


def _kernel(x_hbm, wqkv_hbm, wo_hbm, wr_hbm, wg_hbm, wu_hbm, wd_hbm, out_hbm,
            x_v, wq_v, wk_v, wv_v, wo_v, wr_v, wg_v, wu_v, wd_v,
            wop_v, wgn_v, wun_v, wqvt_v, k_v, vt_v, xn_v, qt_v, out_v, r_v, s0_v, s1_v,
            sem_x, sem_w, sem_o):
    def x_copy(c):
        return pltpu.make_async_copy(x_hbm.at[pl.ds(c * T, T)], x_v.at[pl.ds(c * T, T)], sem_x.at[c])

    def out_copy(c):
        return pltpu.make_async_copy(out_v.at[pl.ds(c * T, T)], out_hbm.at[pl.ds(c * T, T)], sem_o.at[c])

    c_wq = pltpu.make_async_copy(wqkv_hbm.at[:, pl.ds(0, D)], wq_v, sem_w.at[0])
    c_wk = pltpu.make_async_copy(wqkv_hbm.at[:, pl.ds(D, D)], wk_v, sem_w.at[7])
    c_wv = pltpu.make_async_copy(wqkv_hbm.at[:, pl.ds(2 * D, D)], wv_v, sem_w.at[8])
    c_wr = pltpu.make_async_copy(wr_hbm, wr_v, sem_w.at[1])
    c_wo = pltpu.make_async_copy(wo_hbm, wo_v, sem_w.at[2])
    c_wg = pltpu.make_async_copy(wg_hbm, wg_v, sem_w.at[3])
    c_wu = pltpu.make_async_copy(wu_hbm, wu_v, sem_w.at[4])
    c_wd = pltpu.make_async_copy(wd_hbm, wd_v, sem_w.at[5])

    x_copy(0).start()
    c_wk.start()

    k_v[:, 0:2 * T, :] = jnp.zeros((NG, 2 * T, T), BF)
    vt_v[0:2] = jnp.zeros((2, D, T), BF)

    s_refs = (s0_v, s1_v)
    ffn = {}

    def row0(u):
        return u * T if isinstance(u, int) else pl.multiple_of(u * T, T)

    def ln(u, wait):
        r0 = row0(u)
        if wait:
            x_copy(u).wait()
        xf = x_v[pl.ds(r0, T), :].astype(F32)
        mean = jnp.mean(xf, axis=-1, keepdims=True)
        cen = xf - mean
        var = jnp.mean(cen * cen, axis=-1, keepdims=True)
        m_b = _rb(mean)
        v_b = _rb(var)
        s_b = _rb(jnp.sqrt(_rb(v_b + EPS_BF)))
        xn = (_rb(xf - m_b) / s_b).astype(BF)
        xn_v[pl.ds(r0, T), :] = xn

    def proj_k(u, nt):
        r0 = row0(u)
        xn = xn_v[pl.ds(r0, nt * T), :]
        k = _nn(xn, wk_v[...]).astype(BF)
        for g in range(NG):
            k_v[g, pl.ds(r0 + 2 * T, nt * T), :] = k[:, g * 128:(g + 1) * 128]

    def store_qt(u, q):
        qb = (q * QSCALE).astype(BF)
        parts = []
        for h in range(H):
            blk = qb[h * DH:(h + 1) * DH]
            parts.append(pltpu.roll(blk, 64, axis=1) if h % 2 else blk)
        qb = jnp.concatenate(parts, axis=0)
        hrow = lax.broadcasted_iota(jnp.int32, (D, T), 0) >> 4
        half = lax.broadcasted_iota(jnp.int32, (D, T), 1) >> 6
        keep0 = ((hrow ^ half) & 1) == 0
        zero = jnp.zeros((D, T), BF)
        qt_v[u, 0] = jnp.where(keep0, qb, zero)
        qt_v[u, 1] = jnp.where(keep0, zero, qb)

    def proj_qv(u, nt):
        xn = xn_v[pl.ds(row0(u), nt * T), :]
        t = _nt(wqvt_v[...], xn)
        for j in range(nt):
            tj = t[:, j * T:(j + 1) * T]
            store_qt(u + j, tj[0:D])
            vt_v[u + 2 + j] = tj[D:2 * D].astype(BF)
            r_v[u + j] = _rb(tj[2 * D:2 * D + 8])

    def proj_q(u, nt):
        xn = xn_v[pl.ds(row0(u), nt * T), :]
        t = _nt(wqvt_v[0:D], xn)
        for j in range(nt):
            store_qt(u + j, t[:, j * T:(j + 1) * T])

    def proj_v(u, nt):
        xn = xn_v[pl.ds(row0(u), nt * T), :]
        t = _nt(wqvt_v[D:2 * D + 16], xn)
        for j in range(nt):
            tj = t[:, j * T:(j + 1) * T]
            vt_v[u + 2 + j] = tj[0:D].astype(BF)
            r_v[u + j] = _rb(tj[D:D + 8])

    def transpose_w(w_ref, j):
        for i in range(NG):
            wqvt_v[j * D + i * 128: j * D + (i + 1) * 128, :] = w_ref[:, i * 128:(i + 1) * 128].T

    def qk_phase(u, r0, n, nblk, tri_a, tri_e, slot):
        g, par = divmod(n, 2)
        zero = jnp.zeros((16, 128), BF)
        tiles = []
        for p in range(4):
            both = qt_v[u, par, (g * 8 + 2 * p) * 16:(g * 8 + 2 * p + 2) * 16, :]
            rows = [zero] * (2 * p) + [both] + [zero] * (6 - 2 * p)
            tiles.append(jnp.concatenate(rows, axis=0))
        qm = jnp.concatenate(tiles, axis=1)
        skip = 5 - nblk
        ks = r0 + 64 * par + 64 * skip
        kb = k_v[g, pl.ds(ks, 64 * nblk), :]
        s = _nn(kb, qm)
        blocks = [s[64 * b:64 * (b + 1)] for b in range(nblk)]
        lsl = [slice(p * 128, (p + 1) * 128) for p in range(4)]
        if nblk == 5:
            comb = jnp.concatenate([jnp.where(tri_a, blocks[0][:, l_], blocks[4][:, l_]) for l_ in lsl], axis=1)
            mids = blocks[1:4]
        else:
            comb = jnp.concatenate([jnp.where(tri_e, blocks[-1][:, l_], NEG) for l_ in lsl], axis=1)
            mids = blocks[:-1]
        s_ref = s_refs[slot % 2]
        s_ref[0:64, :] = comb
        m = comb
        for i, b in enumerate(mids):
            s_ref[64 * (i + 1):64 * (i + 2), :] = b
            m = jnp.maximum(m, b)
        return jnp.max(m, axis=0, keepdims=True)

    def smpv_phase(u, n, nblk, m, tri_a, slot):
        g, par = divmod(n, 2)
        s_ref = s_refs[slot % 2]
        skip = 5 - nblk
        outs = []
        for p in range(4):
            ls = slice(p * 128, (p + 1) * 128)
            mp = m[:, ls]
            hrow = (g * 8 + 2 * p) * DH
            if nblk == 5:
                ex = lambda b: jnp.exp2(s_ref[64 * b:64 * (b + 1), ls] - mp)
                z = jnp.zeros((64, 128), F32)
                pc = ex(0)
                l = pc
                pa = jnp.where(tri_a, pc, 0.0)
                pe = jnp.where(tri_a, 0.0, pc)
                if par == 0:
                    b1 = ex(1)
                    l = l + b1
                    t0 = jnp.concatenate([pa, b1], axis=0).astype(BF)
                    o = _nn(vt_v[u, hrow:hrow + 32, :], t0)
                    b2 = ex(2)
                    b3 = ex(3)
                    l = l + b2 + b3
                    t1 = jnp.concatenate([b2, b3], axis=0).astype(BF)
                    o = o + _nn(vt_v[u + 1, hrow:hrow + 32, :], t1)
                    t2 = jnp.concatenate([pe, z], axis=0).astype(BF)
                    o = o + _nn(vt_v[u + 2, hrow:hrow + 32, :], t2)
                else:
                    t0 = jnp.concatenate([z, pa], axis=0).astype(BF)
                    o = _nn(vt_v[u, hrow:hrow + 32, :], t0)
                    b1 = ex(1)
                    b2 = ex(2)
                    l = l + b1 + b2
                    t1 = jnp.concatenate([b1, b2], axis=0).astype(BF)
                    o = o + _nn(vt_v[u + 1, hrow:hrow + 32, :], t1)
                    b3 = ex(3)
                    l = l + b3
                    t2 = jnp.concatenate([b3, pe], axis=0).astype(BF)
                    o = o + _nn(vt_v[u + 2, hrow:hrow + 32, :], t2)
                l = jnp.sum(l, axis=0, keepdims=True)
            else:
                ps = [jnp.exp2(s_ref[64 * b:64 * (b + 1), ls] - mp) for b in range(nblk)]
                l = ps[0]
                for b in ps[1:]:
                    l = l + b
                l = jnp.sum(l, axis=0, keepdims=True)
                z = jnp.zeros((64, 128), F32)
                seq = ps[1:] + [ps[0]]
                al = [z] * skip + seq + [z] if par == 0 else [z] * (1 + skip) + seq
                j0 = skip // 2 if par == 0 else (1 + skip) // 2
                P = jnp.concatenate(al[2 * j0:], axis=0).astype(BF)
                vwin = jnp.concatenate([vt_v[u + j, hrow:hrow + 32, :] for j in range(j0, 3)], axis=1)
                o = _nn(vwin, P)
            r = pl.reciprocal(l, approx=True)
            r = r * (2.0 - l * r)
            outs.append(o * r)
        return outs

    def step(u0, nblks, nxt, order):
        lane = lax.broadcasted_iota(jnp.int32, (64, 128), 1)
        row = lax.broadcasted_iota(jnp.int32, (64, 128), 0)
        qi = lane & 63
        tri_a = row > qi
        tri_e = row <= qi
        lane_lo16 = lax.broadcasted_iota(jnp.int32, (16, 128), 1) < 64
        ms, res, ots = {}, {}, {}

        for tk in order.split():
            kind = tk.rstrip('0123456789')
            num = int(tk[len(kind):]) if len(tk) > len(kind) else None
            if kind == 'ln':
                if nxt:
                    for j in range(TP):
                        ln(u0 + TP + j, False)
            elif kind == 'pk':
                if nxt:
                    proj_k(u0 + TP, TP) if num is None else proj_k(u0 + TP + num, 1)
            elif kind == 'pqv':
                if nxt:
                    proj_qv(u0 + TP, TP) if num is None else proj_qv(u0 + TP + num, 1)
            elif kind == 'q':
                j, n = divmod(num, 8)
                ms[num] = qk_phase(u0 + j, row0(u0 + j), n, nblks[j][n % 2], tri_a, tri_e, num)
            elif kind == 's':
                j, n = divmod(num, 8)
                res[num] = smpv_phase(u0 + j, n, nblks[j][n % 2], ms[num], tri_a, num)
            elif kind == 'pw':
                for h in range(H):
                    dst = (h % 2) * (D // 2) + (h // 2) * DH
                    wop_v[dst:dst + DH, :] = wo_v[h * DH:(h + 1) * DH, :]
            elif kind == 'a':
                pe_, po_ = [], []
                for p in range(4):
                    re_, ro_ = res[2 * num][p], res[2 * num + 1][p]
                    pe_.append(jnp.where(lane_lo16, re_[0:16], ro_[0:16]))
                    po_.append(jnp.where(lane_lo16, ro_[16:32], re_[16:32]))
                ots[num] = (jnp.concatenate(pe_, axis=0).astype(BF), jnp.concatenate(po_, axis=0).astype(BF))
            elif kind == 'wo':
                js = range(TP) if num is None else [num]

                def lhs(parity):
                    return jnp.concatenate(
                        [jnp.concatenate([ots[NG * j + g][parity] for g in range(NG)], axis=0).T for j in js], axis=0)
                ae = _nn(lhs(0), wop_v[0:D // 2])
                ao = _nn(lhs(1), wop_v[D // 2:D])
                sw = []
                for i_ in range(len(js)):
                    sw += [ao[i_ * T + 64:(i_ + 1) * T], ao[i_ * T:i_ * T + 64]]
                a = ae + jnp.concatenate(sw, axis=0)
                for i_, j in enumerate(js):
                    r0 = row0(u0 + j)
                    resid = (x_v[pl.ds(r0, T), :].astype(F32) + xn_v[pl.ds(r0, T), :].astype(F32)
                             + a[i_ * T:(i_ + 1) * T])
                    if 'y' in ffn:
                        rows_abs = lax.broadcasted_iota(jnp.int32, (T, D), 0) + (u0 + j) * T
                        resid = resid + jnp.where(rows_abs == ffn['idx'], ffn['y'][0:1, :], 0.0)
                    out_v[pl.ds(r0, T), :] = resid.astype(BF)
                    out_copy(u0 + j).start()
            elif kind in ('fg', 'fu'):
                src, dst = (wg_v, wgn_v) if kind == 'fg' else (wu_v, wun_v)
                for i in range(pl.cdiv(F, 128)):
                    n_ = min(128, F - i * 128)
                    dst[:, i * 128:i * 128 + n_] = src[i * 128:i * 128 + n_, :].T
            elif kind == 'fa':
                r = r_v[...][:, 0, :]
                tok = (lax.broadcasted_iota(jnp.int32, (NT, 128), 0) * 128
                       + lax.broadcasted_iota(jnp.int32, (NT, 128), 1))
                rmax = jnp.max(jnp.max(r, axis=1, keepdims=True), axis=0, keepdims=True)
                idx = jnp.minimum(jnp.min(jnp.where(r == rmax, tok, S)), S - 1)
                blk = pl.multiple_of((idx // 16) * 16, 16)
                sel = (lax.broadcasted_iota(jnp.int32, (16, D), 0) + blk) == idx
                xrow = jnp.sum(jnp.where(sel, xn_v[pl.ds(blk, 16), :].astype(F32), 0.0), axis=0, keepdims=True)
                ffn.update(idx=idx, blk=blk, rmax=rmax, xs=jnp.broadcast_to(xrow, (16, D)).astype(BF))
            elif kind == 'fb':
                ffn['gp'] = _rb(_nn(ffn['xs'], wgn_v[...]))
                ffn['up'] = _rb(_nn(ffn['xs'], wun_v[...]))
            elif kind == 'fc':
                gp = ffn['gp']
                hh = (_rb(gp * jax.nn.sigmoid(gp)) * ffn['up']).astype(BF)
                y = _rb(_nn(hh, wd_v[...]))
                ffn['y'] = _rb(y * _rb(jax.nn.sigmoid(ffn['rmax'])))
            elif kind == 'fd':
                pblk = pl.multiple_of(jnp.minimum(ffn['blk'], u0 * T - 16), 16)
                psel = (lax.broadcasted_iota(jnp.int32, (16, D), 0) + pblk) == ffn['idx']
                cur = out_v[pl.ds(pblk, 16), :].astype(F32)
                out_v[pl.ds(pblk, 16), :] = jnp.where(psel, cur + ffn['y'], cur).astype(BF)
                patch = pltpu.make_async_copy(out_v.at[pl.ds(pblk, 16)], out_hbm.at[pl.ds(pblk, 16)], sem_w.at[6])
                patch.start()
                ffn['patch'] = patch
            else:
                raise ValueError(tk)

    x_copy(0).wait()
    c_wq.start()
    x_copy(1).start()
    ln(0, False)
    c_wk.wait()
    c_wv.start()
    c_wr.start()
    proj_k(0, 1)
    ln(1, True)
    proj_k(1, 1)
    c_wq.wait()
    for c in range(2, 2 + TP):
        x_copy(c).start()
    transpose_w(wq_v, 0)
    proj_q(0, 1)
    c_wv.wait()
    c_wr.wait()
    c_wo.start()
    proj_q(1, 1)
    transpose_w(wv_v, 1)
    wqvt_v[2 * D:2 * D + 16, :] = jnp.broadcast_to(wr_v[...].reshape(1, D), (16, D))
    proj_v(0, TP)
    c_wo.wait()
    for c in range(2, 2 + TP):
        x_copy(c).wait()
    for c in range(2 + TP, NT):
        x_copy(c).start()

    step(0, [(1, 2), (3, 4)], True, ORDER_FIRST)
    c_wg.start()
    c_wu.start()
    c_wd.start()
    for c in range(2 + TP, NT):
        x_copy(c).wait()
    full = [(5, 5)] * TP

    def body(i, carry):
        step((i + 1) * TP, full, True, ORDER_LOOP)
        return carry
    lax.fori_loop(0, NT // TP - 2, body, 0)

    c_wg.wait()
    c_wu.wait()
    c_wd.wait()
    for c in range(NT - TP):
        out_copy(c).wait()
    step(NT - TP, full, False, ORDER_LAST)
    for j in range(TP):
        out_copy(NT - TP + j).wait()
    ffn['patch'].wait()


@jax.jit
def pallas_parallel_sum__sliding_block__moe_arch_mod__prompt_kernel(
    A_x: jax.Array,
    A_wqkv: jax.Array,
    A_wo: jax.Array,
    B_x: jax.Array,
    B_w_r: jax.Array,
    B_w_gate: jax.Array,
    B_w_up: jax.Array,
    B_w_down: jax.Array,
):
    del B_x
    hbm = pl.BlockSpec(memory_space=pltpu.HBM)
    out = pl.pallas_call(
        _kernel,
        out_shape=jax.ShapeDtypeStruct((S, D), BF),
        in_specs=[hbm] * 7,
        out_specs=hbm,
        scratch_shapes=[
            pltpu.VMEM((S, D), BF),
            pltpu.VMEM((D, D), BF),
            pltpu.VMEM((D, D), BF),
            pltpu.VMEM((D, D), BF),
            pltpu.VMEM((D, D), BF),
            pltpu.VMEM((D,), BF),
            pltpu.VMEM((F, D), BF),
            pltpu.VMEM((F, D), BF),
            pltpu.VMEM((F, D), BF),
            pltpu.VMEM((D, D), BF),
            pltpu.VMEM((D, F), BF),
            pltpu.VMEM((D, F), BF),
            pltpu.VMEM((2 * D + 16, D), BF),
            pltpu.VMEM((NG, S + 2 * T, 128), BF),
            pltpu.VMEM((NT + 2, D, T), BF),
            pltpu.VMEM((S, D), BF),
            pltpu.VMEM((NT, 2, D, T), BF),
            pltpu.VMEM((S, D), BF),
            pltpu.VMEM((NT, 8, T), F32),
            pltpu.VMEM((256, 512), F32),
            pltpu.VMEM((256, 512), F32),
            pltpu.SemaphoreType.DMA((NT,)),
            pltpu.SemaphoreType.DMA((9,)),
            pltpu.SemaphoreType.DMA((NT,)),
        ],
        compiler_params=pltpu.CompilerParams(
            vmem_limit_bytes=64 * 1024 * 1024,
            flags={'XLA_TPU_EVENLY_DISTRIBUTE_CRITICAL_NODES': True},
        ),
    )(A_x.reshape(S, D), A_wqkv, A_wo, B_w_r, B_w_gate.T, B_w_up.T, B_w_down)
    return out.reshape(1, S, D)
```
